```python
import os as _os
_os.environ.setdefault("JAX_PLATFORMS", "cpu")
import jax
import jax.numpy as jnp

def _softmax(x, axis=-1):
    return jax.nn.softmax(x, axis=axis)
def _gelu(x):
    return jax.nn.gelu(x, approximate=True)
def _silu(x):
    return jax.nn.silu(x)
def _sigmoid(x):
    return jax.nn.sigmoid(x)
def _layernorm(x, axis=-1, eps=1e-5):
    m = jnp.mean(x, axis=axis, keepdims=True)
    v = jnp.var(x, axis=axis, keepdims=True)
    return (x - m) / jnp.sqrt(v + eps)
def _scatter_add(tgt, idx, src, axis=0):
    return tgt.at[idx].add(src)
def _segment_sum(src, seg, n):
    return jax.ops.segment_sum(src, seg, n)
class _Rng:
    def __init__(self, key):
        self._k = key
    def _next(self):
        self._k, sub = jax.random.split(self._k)
        return sub
    def normal(self, shape):
        return jax.random.normal(self._next(), shape, dtype=jnp.bfloat16)
    def randint(self, lo, hi, shape):
        return jax.random.randint(self._next(), shape, lo, hi, dtype=jnp.int32)
    def uniform(self, shape, lo=0.0, hi=1.0):
        return jax.random.uniform(self._next(), shape, jnp.bfloat16, lo, hi)
    def permutation(self, n):
        return jax.random.permutation(self._next(), n)


kernel_name = 'recurrent_scan__grouped_kv_mqa__mixer_s_mlp__prompt'

def setup_inputs():
    _rng = _Rng(jax.random.key(int.from_bytes(__import__("os").urandom(4), "little")))
    _w = (lambda a: (lambda t: t.astype(jnp.bfloat16) if jnp.issubdtype(t.dtype, jnp.floating) else t)(jnp.asarray(a)))
    def _A_setup():
        B, S, D, H = 1, 2048, 512, 32
        Dh = D // H
        return {
            "x": _w((lambda *s: _rng.normal(s) * 0.05)(B, S, D)),
            "wq": _w((lambda *s: _rng.normal(s) * 0.05)(D, H * Dh)),
            "wk": _w((lambda *s: _rng.normal(s) * 0.05)(D, Dh)),
            "wv": _w((lambda *s: _rng.normal(s) * 0.05)(D, Dh)),
            "wo": _w((lambda *s: _rng.normal(s) * 0.05)(H * Dh, D)),
        }
    _A_in = _A_setup()

    def _B_setup():
        B, S, D, F = 1, 2048, 512, 1792
        return {
            "x":  _w((lambda *s: _rng.normal(s) * 0.05)(B, S, D)),
            "w1": _w((lambda *s: _rng.normal(s) * 0.8)(D, D) * (D ** -0.5)),
            "w2": _w((lambda *s: _rng.normal(s) * 0.8)(D, D) * (D ** -0.5)),
            "w3": _w((lambda *s: _rng.normal(s) * 0.8)(D, F) * (D ** -0.5)),
            "w4": _w((lambda *s: _rng.normal(s) * 0.8)(F, D) * (F ** -0.5)),
        }
    _B_in = _B_setup()

    return {
        "A_x": _A_in["x"],
        "A_wq": _A_in["wq"],
        "A_wk": _A_in["wk"],
        "A_wv": _A_in["wv"],
        "A_wo": _A_in["wo"],
        "B_x": _B_in["x"],
        "B_w1": _B_in["w1"],
        "B_w2": _B_in["w2"],
        "B_w3": _B_in["w3"],
        "B_w4": _B_in["w4"],
    }

def reference(A_x, A_wq, A_wk, A_wv, A_wo, B_x, B_w1, B_w2, B_w3, B_w4):
    def _A_ref(x, wq, wk, wv, wo):
        B, S, D = x.shape
        H = 32
        Dh = D // H
        q = (lambda x, *d: x.transpose(*d))((x @ wq).reshape(B, S, H, Dh), 0, 2, 1, 3)
        k = x @ wk
        v = x @ wv
        scores = jnp.einsum("bhqd,bkd->bhqk", q, k) * (Dh ** -0.5)
        p = _softmax(scores, axis=-1)
        o = jnp.einsum("bhqk,bkd->bhqd", p, v)
        return (lambda x, *d: x.transpose(*d))(o, 0, 2, 1, 3).reshape(B, S, H * Dh) @ wo

    def _B_ref(x, w1, w2, w3, w4):
        B, S, D = x.shape
        h = _gelu(_layernorm(x, axis=-1) @ w1)
        c = D // 4
        g0 = jnp.pad(h[:, :, 0*c:1*c], ((0, 0), (1, 0), (0, 0)))[:, :S, :]
        g1 = jnp.pad(h[:, :, 1*c:2*c], ((0, 0), (0, 1), (0, 0)))[:, 1:, :]
        g2 = jnp.pad(h[:, :, 2*c:3*c], ((0, 0), (2, 0), (0, 0)))[:, :S, :]
        g3 = jnp.pad(h[:, :, 3*c:   ], ((0, 0), (0, 2), (0, 0)))[:, 2:, :]
        hs = jnp.concatenate([g0, g1, g2, g3], axis=-1) @ w2
        x1 = x + hs
        h2 = _gelu(_layernorm(x1, axis=-1) @ w3) @ w4
        return x1 + h2

    x = A_x
    xn = _layernorm(x, axis=-1)
    s = _A_ref(xn, A_wq, A_wk, A_wv, A_wo)
    g = _silu(_B_ref(xn, B_w1, B_w2, B_w3, B_w4))
    return x + s * g
```

```python
import math

import jax
import jax.numpy as jnp
from jax import lax
import jax.experimental.pallas as pl
import jax.experimental.pallas.tpu as pltpu

S, D, H, DH, F = 2048, 512, 32, 16, 1792
BQ = 512
CK = 128
RC = 512
PR = 128
MR = 256
ER = 256
HALO = 8
PA = (2, 4, 14, 160, 80, 1, 1.21)
PB = (1, 5, 14, 160, 80, 1, 1.01)
PM = (2, 8, 160, 80, 1, 1.04)
PL = (1, 3, 9, 12)
VK_MAX = 160
EPS = 1e-5
QSCALE = (DH ** -0.5) * math.log2(math.e)
F32, BF16 = jnp.float32, jnp.bfloat16


def _ln(x):
    m = jnp.mean(x, axis=-1, keepdims=True)
    xc = x - m
    v = jnp.mean(xc * xc, axis=-1, keepdims=True)
    return xc * lax.rsqrt(v + EPS)


def _gelu(x):
    c = math.sqrt(2.0 / math.pi)
    inner = x * (c + (c * 0.044715) * (x * x))
    return x * (0.5 + 0.5 * jnp.tanh(inner))


def _silu(x):
    return x * (0.5 + 0.5 * jnp.tanh(0.5 * x))


def _dot(a, b):
    return jnp.dot(a, b, preferred_element_type=F32)


def _rows(i, n):
    return pl.ds(pl.multiple_of(i * n, n), n)


def _kernel(x_hbm, wq_hbm, wk_hbm, wv_hbm, wo_hbm, w1_hbm, w2_hbm, w3_hbm, w4_hbm,
            out_hbm,
            x_v, wq_v, wk_v, wv_v, wo_v, w1_v, w2_v, w3_v, w4_v,
            wkv_v, xn_v, k_v, vt_v, qt_v, ot_v, h_v, x1n_v, acc_v, s_v, out_v, kb_v, l_v,
            sem_x, sem_w, sem_o):
    nrc = S // RC
    nc = S // CK
    nq = BQ // 128
    ppb = BQ // PR
    n_steps = (S // BQ) * H
    n_pre = S // PR

    def x_copy(i):
        return pltpu.make_async_copy(x_hbm.at[pl.ds(i * RC, RC)], x_v.at[pl.ds(i * RC, RC)], sem_x.at[i])

    def o_copy(i):
        return pltpu.make_async_copy(out_v.at[pl.ds(i * ER, ER)], out_hbm.at[pl.ds(i * ER, ER)], sem_o.at[i])

    w_pairs = [(wk_hbm, wk_v), (wv_hbm, wv_v), (wq_hbm, wq_v), (w1_hbm, w1_v),
               (w2_hbm, w2_v), (w3_hbm, w3_v), (w4_hbm, w4_v), (wo_hbm, wo_v)]
    w_copies = [pltpu.make_async_copy(a, b, sem_w.at[i]) for i, (a, b) in enumerate(w_pairs)]

    x_copy(0).start()
    for c in w_copies[:2]:
        c.start()
    for i in range(1, nrc):
        x_copy(i).start()

    h_v[0:HALO, :] = jnp.zeros((HALO, D), F32)
    h_v[HALO + S:, :] = jnp.zeros((HALO, D), F32)

    w_copies[0].wait()
    w_copies[1].wait()
    wkv_v[...] = jnp.concatenate(
        [wk_v[...].astype(F32), wv_v[...].astype(F32), jnp.zeros((128 - 2 * DH, D), F32)],
        axis=0).T.astype(BF16)

    def kv_chunk(i):
        kv = _dot(xn_v[i * RC:(i + 1) * RC, :], wkv_v[...])
        k_v[i * RC // 2:(i + 1) * RC // 2, :] = pltpu.bitcast(kv.astype(BF16), jnp.uint32)
        vt_v[i] = kv.T[DH:2 * DH, :].astype(BF16)
        if i == 0:
            kf = kv[:VK_MAX].astype(BF16).astype(F32)
            for d in range(DH):
                kb_v[d] = jnp.broadcast_to(kf[:, d:d + 1], (VK_MAX, 128))

    for i in range(nrc):
        x_copy(i).wait()
        if i == 1:
            for c in w_copies[2:4]:
                c.start()
        if i == nrc - 1:
            for c in w_copies[4:]:
                c.start()
        if i > 0:
            kv_chunk(i - 1)
        xn_v[i * RC:(i + 1) * RC, :] = _ln(x_v[i * RC:(i + 1) * RC, :].astype(F32)).astype(BF16)

    def q_piece(i):
        q = _dot(xn_v[_rows(i, PR), :], wq_v[...]) * QSCALE
        qt_v[i] = q.T.astype(BF16)

    def h_piece(i):
        xnn = _ln(xn_v[_rows(i, PR), :].astype(F32)).astype(BF16)
        h_v[pl.ds(pl.multiple_of(i * PR + HALO, 8), PR), :] = _gelu(_dot(xnn, w1_v[...]))

    def x1_piece(i):
        r0 = pl.multiple_of(i * PR, PR)
        c = D // 4
        parts = []
        for g, sh in enumerate((1, -1, 2, -2)):
            hb = h_v[pl.ds(r0, PR + 2 * HALO), g * c:(g + 1) * c]
            parts.append(hb[HALO - sh:HALO - sh + PR])
        hs = _dot(jnp.concatenate(parts, axis=1).astype(BF16), w2_v[...])
        x1 = xn_v[_rows(i, PR), :].astype(F32) + hs
        acc_v[_rows(i, PR), :] = x1
        x1n_v[_rows(i, PR // 2), :] = pltpu.bitcast(_ln(x1).astype(BF16), jnp.uint32)

    def mlp_pieces(i):
        nr = S // MR
        r = i & (nr - 1)
        f0 = pl.multiple_of(lax.shift_right_logical(i, nr.bit_length() - 1) * 128, 128)
        hid = []

        def up():
            a = pltpu.bitcast(x1n_v[_rows(r, MR // 2), :], BF16)
            hid.append(_gelu(_dot(a, w3_v[:, pl.ds(f0, 128)])).astype(BF16))

        def down():
            acc_v[_rows(r, MR), :] += _dot(hid[0], w4_v[pl.ds(f0, 128), :])

        return up, down

    def out_piece(j, e):
        inv = l_v[_rows(j, H * 8), e * ER:(e + 1) * ER].reshape(H, 8, ER)
        inv = jnp.concatenate([inv, inv], axis=1)
        o = ot_v[_rows(j, D), e * ER:(e + 1) * ER].reshape(H, DH, ER) * inv
        o = o.reshape(D, ER).T.astype(BF16)
        sv = _dot(o, wo_v[...])
        rows = _rows(j * (BQ // ER) + e, ER)
        out_v[rows, :] = (x_v[rows, :].astype(F32) + sv * _silu(acc_v[rows, :])).astype(BF16)

    def get_q(t):
        j = lax.shift_right_logical(t, 5)
        r = pl.multiple_of(lax.shift_left(t & (H - 1), 4), DH)
        return jnp.concatenate([qt_v[j * ppb + u, pl.ds(r, DH), :] for u in range(ppb)], axis=1)

    def qk_mxu(q, lo, hi):
        kk = pltpu.bitcast(k_v[lo // 2:hi // 2, :], BF16)
        s = _dot(kk[:, :DH], q)
        s_v[lo:hi, :] = s
        return jnp.max(s.reshape((hi - lo) // 8, 8, BQ), axis=0)

    def qk_vpu(q, j, lo, hi, after):
        lanes = slice(j * 128, (j + 1) * 128)
        never = after[0:8, lanes] > jnp.inf
        qq = q[:, lanes].astype(F32)
        qq = jnp.concatenate([jnp.where(never, 0.0, qq[:8]), jnp.where(never, 0.0, qq[8:])], axis=0)
        s = None
        for d in range(DH):
            e = kb_v[d, lo:hi, :] * qq[d:d + 1, :]
            s = e if s is None else s + e
        s_v[lo:hi, lanes] = s
        return jnp.max(s.reshape((hi - lo) // 8, 8, 128), axis=0)

    def mx(a, b):
        return b if a is None else jnp.maximum(a, b)

    def step(t, m8, extra, plan=None):
        m_cur = jnp.max(m8, axis=0, keepdims=True)
        if plan:
            gap, late_from, vk, vg, v0, vs = plan
            q = get_q(t + 1)
            pieces = [(j, g) for j in range(nq) for g in range(vk // vg)]
            slots = [min(v0 + int(i * vs), nc - 1) for i in range(len(pieces))]
        ss = [s_v[c * CK:(c + 1) * CK, :] for c in range(nc)]
        m_n = l = acc = None
        mv = [None] * nq
        for c in range(nc):
            p = jnp.exp2(ss[c] - m_cur)
            ll = jnp.sum(p.reshape(CK // 8, 8, BQ), axis=0)
            l = ll if l is None else l + ll
            if plan and c != gap:
                qc = c if c > gap else c + 1
                keys = (max(qc * CK, vk), (qc + 1) * CK)
            if plan and c != gap and c < late_from:
                m_n = mx(m_n, qk_mxu(q, *keys))
            if c in extra:
                extra[c]()
            kc = c * CK
            a = _dot(vt_v[kc // RC, :, kc % RC:kc % RC + CK], p.astype(BF16))
            acc = a if acc is None else acc + a
            if plan and c >= late_from:
                m_n = mx(m_n, qk_mxu(q, *keys))
            if plan:
                for (j, g), sl in zip(pieces, slots):
                    if sl == c:
                        mv[j] = mx(mv[j], qk_vpu(q, j, g * vg, (g + 1) * vg, acc))
        l_v[_rows(t, 8), :] = jnp.broadcast_to(1.0 / jnp.sum(l, axis=0, keepdims=True), (8, BQ))
        ot_v[_rows(t, DH), :] = acc
        if plan:
            return jnp.maximum(m_n, jnp.concatenate(mv, axis=1))

    def pre_step(t, m, cfg, with_q):
        extra = {cfg[1]: lambda: h_piece(jnp.minimum(t + 1, n_pre - 1)), cfg[2]: lambda: x1_piece(t)}
        if with_q:
            extra[cfg[0]] = lambda: q_piece(t + ppb)
        return step(t, m, extra, cfg[1:])

    def mlp_step(t, m):
        up, down = mlp_pieces(t - n_pre)
        return step(t, m, {PM[0]: up, PM[1]: down}, (PM[0], nc) + PM[2:])

    w_copies[2].wait()
    w_copies[3].wait()
    kv_chunk(nrc - 1)
    for i in range(ppb):
        q_piece(i)
    h_piece(0)
    q0 = get_q(jnp.int32(0))
    m = None
    for c in range(nc):
        m = mx(m, qk_mxu(q0, c * CK, (c + 1) * CK))
    w_copies[4].wait()
    m = lax.fori_loop(0, n_pre - ppb, lambda t, m: pre_step(t, m, PA, True), m)
    m = lax.fori_loop(n_pre - ppb, n_pre, lambda t, m: pre_step(t, m, PB, False), m)
    w_copies[5].wait()
    w_copies[6].wait()
    m = lax.fori_loop(n_pre, n_steps - 1, mlp_step, m)
    w_copies[7].wait()
    up, down = mlp_pieces(jnp.int32(n_steps - 1 - n_pre))
    step(n_steps - 1, m, {PL[0]: up, PL[1]: lambda: out_piece(0, 0), PL[2]: down,
                          PL[3]: lambda: out_piece(0, 1)})

    for e in range(BQ // ER):
        o_copy(e).start()

    for j in range(1, S // BQ):
        for e in range(BQ // ER):
            out_piece(j, e)
            o_copy(j * (BQ // ER) + e).start()
    for i in range(S // ER):
        o_copy(i).wait()


@jax.jit
def pallas_recurrent_scan__grouped_kv_mqa__mixer_s_mlp__prompt_kernel(
    A_x: jax.Array,
    A_wq: jax.Array,
    A_wk: jax.Array,
    A_wv: jax.Array,
    A_wo: jax.Array,
    B_x: jax.Array,
    B_w1: jax.Array,
    B_w2: jax.Array,
    B_w3: jax.Array,
    B_w4: jax.Array,
):
    del B_x
    any_spec = pl.BlockSpec(memory_space=pl.ANY)
    vm = pltpu.VMEM
    out = pl.pallas_call(
        _kernel,
        out_shape=jax.ShapeDtypeStruct((S, D), A_x.dtype),
        in_specs=[any_spec] * 9,
        out_specs=any_spec,
        scratch_shapes=[
            vm((S, D), BF16), vm((D, D), BF16), vm((DH, D), BF16), vm((DH, D), BF16),
            vm((D, D), BF16), vm((D, D), BF16), vm((D, D), BF16), vm((D, F), BF16), vm((F, D), BF16),
            vm((D, 128), BF16),
            vm((S, D), BF16),
            vm((S // 2, 128), jnp.uint32),
            vm((S // RC, DH, RC), BF16),
            vm((S // PR, D, PR), BF16),
            vm((S // BQ * D, BQ), F32),
            vm((S + 2 * HALO, D), F32),
            vm((S // 2, D), jnp.uint32),
            vm((S, D), F32),
            vm((S, BQ), F32),
            vm((S, D), BF16),
            vm((DH, VK_MAX, 128), F32),
            vm((S // BQ * H * 8, BQ), F32),
            pltpu.SemaphoreType.DMA((S // RC,)),
            pltpu.SemaphoreType.DMA((8,)),
            pltpu.SemaphoreType.DMA((S // ER,)),
        ],
        compiler_params=pltpu.CompilerParams(
            vmem_limit_bytes=100 * 1024 * 1024,
            flags={"XLA_TPU_EVENLY_DISTRIBUTE_CRITICAL_NODES": True}),
        name="fused_mqa_mixer",
    )(A_x.reshape(S, D), A_wq, A_wk.T, A_wv.T, A_wo, B_w1, B_w2, B_w3, B_w4)
    return out.reshape(1, S, D)
```
